```python
import os as _os
_os.environ.setdefault("JAX_PLATFORMS", "cpu")
import jax
import jax.numpy as jnp

def _softmax(x, axis=-1):
    return jax.nn.softmax(x, axis=axis)
def _gelu(x):
    return jax.nn.gelu(x, approximate=True)
def _silu(x):
    return jax.nn.silu(x)
def _sigmoid(x):
    return jax.nn.sigmoid(x)
def _layernorm(x, axis=-1, eps=1e-5):
    m = jnp.mean(x, axis=axis, keepdims=True)
    v = jnp.var(x, axis=axis, keepdims=True)
    return (x - m) / jnp.sqrt(v + eps)
def _scatter_add(tgt, idx, src, axis=0):
    return tgt.at[idx].add(src)
def _segment_sum(src, seg, n):
    return jax.ops.segment_sum(src, seg, n)
class _Rng:
    def __init__(self, key):
        self._k = key
    def _next(self):
        self._k, sub = jax.random.split(self._k)
        return sub
    def normal(self, shape):
        return jax.random.normal(self._next(), shape, dtype=jnp.bfloat16)
    def randint(self, lo, hi, shape):
        return jax.random.randint(self._next(), shape, lo, hi, dtype=jnp.int32)
    def uniform(self, shape, lo=0.0, hi=1.0):
        return jax.random.uniform(self._next(), shape, jnp.bfloat16, lo, hi)
    def permutation(self, n):
        return jax.random.permutation(self._next(), n)


kernel_name = 'parallel_sum__mha_block__swiglu_ffn__prompt'

def setup_inputs():
    _rng = _Rng(jax.random.key(int.from_bytes(__import__("os").urandom(4), "little")))
    _w = (lambda a: (lambda t: t.astype(jnp.bfloat16) if jnp.issubdtype(t.dtype, jnp.floating) else t)(jnp.asarray(a)))
    def _A_setup():
        B, S, D, H = 1, 2048, 640, 32
        return {
            "x": _w((lambda *s: _rng.normal(s) * 0.05)(B, S, D)),
            "wqkv": _w((lambda *s: _rng.normal(s) * 0.1)(D, 3 * D)),
            "wo": _w((lambda *s: _rng.normal(s) * 0.05)(D, D)),
        }
    _A_in = _A_setup()

    def _B_setup():
        B, S, D, F = 1, 2048, 640, 1536
        return {
            "x": _w((lambda *s: _rng.normal(s) * 0.05)(B, S, D)),
            "w_gate": _w((lambda *s: _rng.normal(s) * 0.05)(D, F)),
            "w_up": _w((lambda *s: _rng.normal(s) * 0.05)(D, F)),
            "w_down": _w((lambda *s: _rng.normal(s) * 0.05)(F, D)),
        }
    _B_in = _B_setup()

    return {
        "A_x": _A_in["x"],
        "A_wqkv": _A_in["wqkv"],
        "A_wo": _A_in["wo"],
        "B_x": _B_in["x"],
        "B_w_gate": _B_in["w_gate"],
        "B_w_up": _B_in["w_up"],
        "B_w_down": _B_in["w_down"],
    }

def reference(A_x, A_wqkv, A_wo, B_x, B_w_gate, B_w_up, B_w_down):
    def _A_ref(x, wqkv, wo):
        B, S, D = x.shape
        H = 32
        Dh = D // H
        qkv = (lambda x, *d: x.transpose(*d))((x @ wqkv).reshape(B, S, 3, H, Dh), 2, 0, 3, 1, 4)
        q, k, v = qkv[0], qkv[1], qkv[2]
        scores = jnp.einsum("bhqd,bhkd->bhqk", q, k) * (Dh ** -0.5)
        p = _softmax(scores, axis=-1)
        o = jnp.einsum("bhqk,bhkd->bhqd", p, v)
        return (lambda x, *d: x.transpose(*d))(o, 0, 2, 1, 3).reshape(B, S, D) @ wo

    def _B_ref(x, w_gate, w_up, w_down):
        g = _silu(x @ w_gate)
        u = x @ w_up
        return (g * u) @ w_down

    x = A_x
    xn = _layernorm(x, axis=-1)
    return x + _A_ref(xn, A_wqkv, A_wo) + _B_ref(xn, B_w_gate, B_w_up, B_w_down)
```

```python
import math

import jax
import jax.numpy as jnp
from jax import lax
import jax.experimental.pallas as pl
import jax.experimental.pallas.tpu as pltpu

H = 32
LANES = 128
F32 = jnp.float32
BF16 = jnp.bfloat16

TA = 512
TC = 512
CQ = 512
CK = 128
MP = 24

NN = (((1,), (0,)), ((), ()))
NT = (((1,), (1,)), ((), ()))


def _dot(a, b, dims=NN):
    return lax.dot_general(a, b, dims, preferred_element_type=F32)


def _kernel(x_hbm, wqkv_hbm, wo_hbm, wg_hbm, wu_hbm, wd_hbm, out_hbm,
            x_v, wqkv_v, wo_v, wg_v, wu_v, wd_v, out_v,
            wt_s, xn_s, kg_s, qg_s, vt_s, s_s, ot_s, m_s, sems):
    S, D = x_v.shape
    DH = D // H
    G = D // LANES
    na, nc = S // TA, S // TC
    qscale = (DH ** -0.5) * math.log2(math.e)

    def x_copy(c):
        rows = pl.ds(c * TA, TA)
        return pltpu.make_async_copy(x_hbm.at[rows, :], x_v.at[rows, :], sems.at[c])

    def w_copy(p):
        cols = pl.ds(p * D, D)
        return pltpu.make_async_copy(wqkv_hbm.at[:, cols], wqkv_v.at[p], sems.at[na + p])

    late = [pltpu.make_async_copy(src, dst, sems.at[na + 3 + i]) for i, (src, dst) in
            enumerate(((wg_hbm, wg_v), (wu_hbm, wu_v), (wd_hbm, wd_v), (wo_hbm, wo_v)))]

    def out_copy(c):
        rows = pl.ds(c * TC, TC)
        return pltpu.make_async_copy(out_v.at[rows, :], out_hbm.at[rows, :], sems.at[na + 7 + c])

    x_copy(0).start()
    for p in (1, 0, 2):
        w_copy(p).start()
    for c in range(1, na):
        x_copy(c).start()
    for cp in late:
        cp.start()

    def layernorm(c):
        rows = pl.ds(pl.multiple_of(c * TA, TA), TA)
        x = x_v[rows, :].astype(F32)
        mean = jnp.sum(x, axis=-1, keepdims=True) * (1.0 / D)
        xc = x - mean
        var = jnp.sum(xc * xc, axis=-1, keepdims=True) * (1.0 / D)
        xn_s[rows, :] = (xc * lax.rsqrt(var + 1e-5)).astype(BF16)

    def project(c):
        rows = pl.ds(pl.multiple_of(c * TA, TA), TA)
        xn = xn_s[rows, :]
        k = _dot(xn, wqkv_v[1]).astype(BF16)
        lane_hi = lax.broadcasted_iota(jnp.int32, (TA, LANES), 1) >= LANES // 2
        for g in range(G):
            kg = k[:, g * LANES:(g + 1) * LANES]
            kg_s[g, rows, :] = kg
            if g + 1 < G:
                kg_s[G + g, rows, :] = jnp.where(lane_hi, kg, k[:, (g + 1) * LANES:(g + 2) * LANES])
        qt = (_dot(wt_s[0], xn, NT) * qscale).astype(BF16)
        half = LANES // 2
        for g in range(G):
            qg_s[g, :, rows] = qt[g * LANES:(g + 1) * LANES]
            if g + 1 < G:
                qg_s[G + g, 0:half, rows] = qt[(g + 1) * LANES:(g + 1) * LANES + half]
                qg_s[G + g, half:LANES, rows] = qt[g * LANES + half:(g + 1) * LANES]
        vt = _dot(wt_s[1], xn, NT).astype(BF16).astype(F32)
        sub = lax.broadcasted_iota(jnp.int32, (8, TA), 0)
        for h in range(H):
            r0 = (h * DH) // 8 * 8
            if h % 2 == 0:
                vt_s[h, 0:16, rows] = vt[r0:r0 + 16]
                vt_s[h, 16:24, rows] = jnp.where(sub < 4, vt[r0 + 16:r0 + 24], 1.0)
            else:
                vt_s[h, 0:8, rows] = jnp.where(sub >= 4, vt[r0:r0 + 8], 1.0)
                vt_s[h, 8:24, rows] = vt[r0 + 8:r0 + 24]

    x_copy(0).wait()
    layernorm(0)
    for p in (1, 0, 2):
        w_copy(p).wait()
    wt_s[0] = wqkv_v[0].T
    wt_s[1] = wqkv_v[2].T

    def phase_a(c, carry):
        x_copy(c + 1).wait()
        project(c)
        layernorm(c + 1)
        return carry

    lax.fori_loop(0, na - 1, phase_a, 0)
    project(na - 1)

    def head_group(h):
        start = h * DH
        j = start // LANES
        return jnp.where(start % LANES > LANES - DH, G + j, j)

    def masked_q(h, g, qs):
        row = lax.broadcasted_iota(jnp.int32, (LANES // 2, CQ), 0)
        keep = ((row - h * (DH // 2)) & (LANES // 2 - 1)) < DH // 2
        q = pltpu.bitcast(qg_s[g, :, qs], jnp.uint32)
        return pltpu.bitcast(jnp.where(keep, q, jnp.uint32(0)), BF16)

    def attend(qs, h_qk, h_pv):
        if h_qk is not None:
            g = head_group(h_qk)
            q = masked_q(h_qk, g, qs)
            mx = None
        if h_pv is not None:
            m = m_s[:, qs]
            acc = None
        for c in range(S // CK):
            ks = pl.ds(c * CK, CK)
            if h_pv is not None:
                p = jnp.exp2(s_s[ks, qs] - m).astype(BF16)
            if h_qk is not None:
                s = _dot(kg_s[g, ks, :], q)
                s_s[ks, qs] = s
                cm = jnp.max(s.reshape(CK // 8, 8, CQ), axis=0)
                mx = cm if mx is None else jnp.maximum(mx, cm)
            if h_pv is not None:
                o = _dot(vt_s[h_pv, :, ks], p)
                acc = o if acc is None else acc + o
        if h_pv is not None:
            l = jnp.where(h_pv % 2 == 0, acc[MP - 1:MP], acc[0:1])
            ot_s[h_pv, :, qs] = acc * (1.0 / l)
        if h_qk is not None:
            m_s[:, qs] = jnp.max(mx, axis=0, keepdims=True)

    def first_head(j, carry):
        attend(pl.ds(pl.multiple_of(j * CQ, CQ), CQ), 0, None)
        return carry

    lax.fori_loop(0, S // CQ, first_head, 0)

    def head_step(h, carry):
        for j in range(S // CQ):
            attend(pl.ds(j * CQ, CQ), h + 1, h)
        return carry

    lax.fori_loop(0, H - 1, head_step, 0)

    for cp in late:
        cp.wait()

    def phase_c(c, carry):
        rows = pl.ds(pl.multiple_of(c * TC, TC), TC)
        attend(rows, None, H - 1)
        xn = xn_s[rows, :]
        gate = _dot(xn, wg_v[...])
        up = _dot(xn, wu_v[...])
        hid = (gate * jax.nn.sigmoid(gate) * up).astype(BF16)
        y = _dot(hid, wd_v[...])
        sub = lax.broadcasted_iota(jnp.int32, (8, TC), 0)
        parts = []
        for h in range(0, H, 2):
            parts.append(ot_s[h, 0:16, rows])
            parts.append(jnp.where(sub < 4, ot_s[h, 16:24, rows], ot_s[h + 1, 0:8, rows]))
            parts.append(ot_s[h + 1, 8:24, rows])
        o = jnp.concatenate(parts, axis=0).T.astype(BF16)
        y = y + _dot(o, wo_v[...])
        out_v[rows, :] = (x_v[rows, :].astype(F32) + y).astype(out_v.dtype)
        out_copy(c).start()
        return carry

    lax.fori_loop(0, nc, phase_c, 0)
    for c in range(nc):
        out_copy(c).wait()


@jax.jit
def pallas_parallel_sum__mha_block__swiglu_ffn__prompt_kernel(
    A_x, A_wqkv, A_wo, B_x, B_w_gate, B_w_up, B_w_down,
):
    del B_x
    B, S, D = A_x.shape
    F = B_w_gate.shape[1]
    G = D // LANES
    dt = A_x.dtype
    any_spec = pl.BlockSpec(memory_space=pl.ANY)
    out = pl.pallas_call(
        _kernel,
        name="mha_swiglu",
        out_shape=jax.ShapeDtypeStruct((S, D), dt),
        in_specs=[any_spec] * 6,
        out_specs=any_spec,
        scratch_shapes=[
            pltpu.VMEM((S, D), dt),
            pltpu.VMEM((3, D, D), dt),
            pltpu.VMEM((D, D), dt),
            pltpu.VMEM((D, F), dt),
            pltpu.VMEM((D, F), dt),
            pltpu.VMEM((F, D), dt),
            pltpu.VMEM((S, D), dt),
            pltpu.VMEM((2, D, D), BF16),
            pltpu.VMEM((S, D), BF16),
            pltpu.VMEM((2 * G - 1, S, LANES), BF16),
            pltpu.VMEM((2 * G - 1, LANES, S), BF16),
            pltpu.VMEM((H, MP, S), F32),
            pltpu.VMEM((S, S), F32),
            pltpu.VMEM((H, MP, S), F32),
            pltpu.VMEM((1, S), F32),
            pltpu.SemaphoreType.DMA((S // TA + 7 + S // TC,)),
        ],
        compiler_params=pltpu.CompilerParams(vmem_limit_bytes=110 * 2**20),
    )(A_x.reshape(S, D), A_wqkv, A_wo, B_w_gate, B_w_up, B_w_down)
    return out.reshape(B, S, D)
```

```python
import functools
import math

import jax
import jax.numpy as jnp
from jax import lax
import jax.experimental.pallas as pl
import jax.experimental.pallas.tpu as pltpu

H = 32
LANES = 128
F32 = jnp.float32
BF16 = jnp.bfloat16
U32 = jnp.uint32

X_CHUNKS = (320, 512, 512, 704)
OUT_CHUNKS = (256,) * 7 + (128, 128)
TK = 64
TQV = 1024
RQV = 64
CQ = 512
CK = 128
RK = 16
VPU_EVERY = 2
MP = 24
FK = 4

NN = (((1,), (0,)), ((), ()))
NT = (((1,), (1,)), ((), ()))


def _dot(a, b, dims=NN):
    return lax.dot_general(a, b, dims, preferred_element_type=F32)


class _Spread:
    def __init__(self, items, slots):
        self.items, self.slots, self.done, self.tick = list(items), slots, 0, 0

    def step(self, ready=None):
        self.tick += 1
        target = min(len(self.items), -(-len(self.items) * self.tick // self.slots))
        while self.done < target and (ready is None or ready(self.done)):
            self.items[self.done]()
            self.done += 1

    def finish(self):
        assert self.done == len(self.items)


def _kernel(x_hbm, wqkv_hbm, wo_hbm, wg_hbm, wu_hbm, wd_hbm, out_hbm,
            x_v, wqkv_v, wo_v, wg_v, wu_v, wd_v, out_v,
            wt_s, xn_s, kg_s, qg_s, qm_s, qf_s, vt_s, s_s, ot_s, m_s,
            y_s, hid_s, kb_s, sems):
    S, D = out_v.shape
    F = wg_v.shape[1]
    DH = D // H
    G = D // LANES
    TF = S // H
    nx, no, nq, nk = len(X_CHUNKS), len(OUT_CHUNKS), S // CQ, S // CK
    x_off = [sum(X_CHUNKS[:i]) for i in range(nx)]
    out_off = [sum(OUT_CHUNKS[:i]) for i in range(no)]
    q_scale = (DH ** -0.5) * math.log2(math.e)
    vpu_chunks = list(range(0, nk, VPU_EVERY))
    part = functools.partial

    def tile(g, n=1):
        return pl.ds(g * LANES, n * LANES)

    def aligned(start, size):
        return pl.ds(start if isinstance(start, int) else pl.multiple_of(start, size), size)

    def xn_block(i, size):
        return pltpu.bitcast(xn_s[aligned(i * (size // 2), size // 2), :], BF16)

    def x_copy(c):
        rows = pl.ds(x_off[c], X_CHUNKS[c])
        return pltpu.make_async_copy(x_hbm.at[rows, :], x_v.at[rows, :], sems.at[c])

    def w_copy(p):
        return pltpu.make_async_copy(
            wqkv_hbm.at[:, pl.ds(p * D, D)], wqkv_v.at[p], sems.at[nx + p])

    def out_copy(c):
        rows = pl.ds(out_off[c], OUT_CHUNKS[c])
        return pltpu.make_async_copy(
            out_v.at[rows, :], out_hbm.at[rows, :], sems.at[nx + 7 + c])

    late_copies = [
        pltpu.make_async_copy(src, dst, sems.at[nx + 3 + i]) for i, (src, dst) in
        enumerate(((wg_hbm, wg_v), (wu_hbm, wu_v), (wd_hbm, wd_v), (wo_hbm, wo_v)))]

    def layernorm(start, size):
        x = x_v[pl.ds(start, size), :].astype(F32)
        mean = jnp.sum(x, axis=-1, keepdims=True) * (1.0 / D)
        xc = x - mean
        var = jnp.sum(xc * xc, axis=-1, keepdims=True) * (1.0 / D)
        xn = (xc * lax.rsqrt(var + 1e-5)).astype(BF16)
        xn_s[pl.ds(start // 2, size // 2), :] = pltpu.bitcast(xn, U32)

    def project_k(i):
        rows = pl.ds(i * TK // 2, TK // 2)
        upper = lax.broadcasted_iota(jnp.int32, (TK // 2, LANES), 1) >= LANES // 2
        k = pltpu.bitcast(_dot(xn_block(i, TK), wqkv_v[1]).astype(BF16), U32)
        for g in range(G):
            kg = k[:, g * LANES:(g + 1) * LANES]
            kg_s[g, rows, :] = kg
            if g + 1 < G:
                kg_s[G + g, rows, :] = jnp.where(upper, kg, k[:, (g + 1) * LANES:(g + 2) * LANES])

    x_copy(0).start()
    w_copy(1).start()
    x_copy(0).wait()
    x_copy(1).start()
    layernorm(0, X_CHUNKS[0])
    w_copy(1).wait()
    for c in range(2, nx):
        x_copy(c).start()
    for c in range(nx):
        if c:
            x_copy(c).wait()
        if c == 1:
            w_copy(0).start()
            w_copy(2).start()
        if c + 1 == nx:
            w_copy(0).wait()
            w_copy(2).wait()
            for copy in late_copies:
                copy.start()
            for i, p in enumerate((0, 2)):
                wt_s[i] = pltpu.bitcast(wqkv_v[p].T, U32)
        for i in range(x_off[c] // TK, (x_off[c] + X_CHUNKS[c]) // TK):
            if i:
                project_k(i - 1)
            if c:
                layernorm(i * TK, TK)
    project_k(S // TK - 1)

    def head_group(h):
        start = h * DH
        straddles = start % LANES > LANES - DH
        if isinstance(h, int):
            return start // LANES + (G if straddles else 0)
        return jnp.where(straddles, G + start // LANES, start // LANES)

    def stage_q(h, cols, r0, n):
        row = lax.broadcasted_iota(jnp.int32, (n, cols.size), 0) + r0
        keep = ((row - h * (DH // 2)) & (LANES // 2 - 1)) < DH // 2
        rows = pl.ds(r0, n)
        qm_s[rows, cols] = jnp.where(keep, qg_s[head_group(h), rows, cols], U32(0))

    def splat_keys(h, chunk, slot):
        rows = pl.ds(((chunk + 1) * CK - RK) // 2, RK // 2)
        k = pltpu.bitcast(kg_s[head_group(h), rows, :], BF16).astype(F32)
        k = pltpu.roll(k, (LANES - (h * DH) % LANES) % LANES, 1)
        for d in range(DH):
            kb_s[slot, d] = jnp.broadcast_to(k[:, d:d + 1], (RK, LANES))

    def vpu_scores(h, slot, cols):
        acc = None
        for d in range(DH):
            term = kb_s[slot, d] * qf_s[h, pl.ds(d, 1), cols]
            acc = term if acc is None else acc + term
        return acc

    def project_qv(c, carry):
        cols = aligned(c * TQV, TQV)
        xn = xn_block(c, TQV)

        def project(i):
            return jnp.concatenate(
                [_dot(pltpu.bitcast(wt_s[i, r // 2:(r + RQV) // 2], BF16), xn, NT)
                 for r in range(0, D, RQV)], axis=0)

        q = (project(0) * q_scale).astype(BF16)
        qu = pltpu.bitcast(q, U32)
        full, half = LANES // 2, LANES // 4
        for g in range(G):
            qg_s[g, :, cols] = qu[g * full:(g + 1) * full]
            if g + 1 < G:
                qg_s[G + g, 0:half, cols] = qu[(g + 1) * full:(g + 1) * full + half]
                qg_s[G + g, half:full, cols] = qu[g * full + half:(g + 1) * full]
        qf = q.astype(F32)
        for h in range(H):
            qf_s[h, 0:DH, cols] = qf[h * DH:(h + 1) * DH]
        v = project(1).astype(BF16).astype(F32)
        sub = lax.broadcasted_iota(jnp.int32, (8, TQV), 0)
        for h in range(H):
            r0 = (h * DH) // 8 * 8
            if h % 2 == 0:
                vt_s[h, 0:16, cols] = v[r0:r0 + 16]
                vt_s[h, 16:24, cols] = jnp.where(sub < 4, v[r0 + 16:r0 + 24], 1.0)
            else:
                vt_s[h, 0:8, cols] = jnp.where(sub >= 4, v[r0:r0 + 8], 1.0)
                vt_s[h, 8:24, cols] = v[r0 + 8:r0 + 24]
        return carry

    for slot, chunk in enumerate(vpu_chunks):
        splat_keys(0, chunk, slot)
    lax.fori_loop(0, S // TQV, project_qv, 0)
    stage_q(0, pl.ds(0, CQ), 0, LANES // 2)
    for copy in late_copies:
        copy.wait()

    def ffn_pieces(c):
        rows = aligned(c * TF, TF)
        state = {}

        def gate(n):
            state["gate"] = _dot(xn_block(c, TF), wg_v[:, tile(n)])

        def up(n):
            half = 0.5 * state["gate"]
            silu = half + half * jnp.tanh(half)
            hid = (silu * _dot(xn_block(c, TF), wu_v[:, tile(n)])).astype(BF16)
            hid_s[:, tile(n)] = pltpu.bitcast(hid, U32)

        def down(g, n):
            y = _dot(pltpu.bitcast(hid_s[:, tile(n, FK)], BF16), wd_v[tile(n, FK), tile(g)])
            state["y"] = state["y"] + y if n else x_v[rows, tile(g)].astype(F32) + y
            if n + FK == F // LANES:
                y_s[rows, tile(g)] = state["y"]

        pieces = [part(f, n) for n in range(F // LANES) for f in (gate, up)]
        return pieces + [part(down, g, n) for g in range(G) for n in range(0, F // LANES, FK)]

    def attend(q0, h_qk, h_pv, next_keys=None, others=()):
        qs = pl.ds(q0, CQ)
        tiles = CQ // LANES
        top = [None] * tiles
        items, item_chunk = [], []

        def update_max(t, value):
            top[t] = value if top[t] is None else jnp.maximum(top[t], value)

        def vpu_item(slot, chunk, t):
            cols = pl.ds(q0 + t * LANES, LANES)
            s = vpu_scores(h_qk, slot, cols)
            s_s[pl.ds((chunk + 1) * CK - RK, RK), cols] = s
            update_max(t, jnp.maximum(s[0:8], s[8:16]))
            if next_keys is not None and t + 1 == tiles:
                splat_keys(next_keys, chunk, slot)

        if h_qk is not None:
            group = head_group(h_qk)
            q = pltpu.bitcast(qm_s[:, qs], BF16)
            for slot, chunk in enumerate(vpu_chunks):
                for t in range(tiles):
                    items.append(part(vpu_item, slot, chunk, t))
                    item_chunk.append(chunk)
        if h_pv is not None:
            m = m_s[:, qs]
            acc = None
        vpu = _Spread(items, 2 * nk)

        for c in range(nk):
            ks = pl.ds(c * CK, CK)
            if h_pv is not None:
                p = jnp.exp2(s_s[ks, qs].reshape(CK // 8, 8, CQ) - m[None]).reshape(CK, CQ)
            vpu.step(lambda i: item_chunk[i] <= c)
            if h_qk is not None:
                n = CK - RK if c in vpu_chunks else CK
                k = pltpu.bitcast(kg_s[group, pl.ds(c * CK // 2, n // 2), :], BF16)
                s = _dot(k, q)
                s_s[pl.ds(c * CK, n), qs] = s
                block_max = jnp.max(s.reshape(n // 8, 8, CQ), axis=0)
                for t in range(tiles):
                    update_max(t, block_max[:, t * LANES:(t + 1) * LANES])
            vpu.step(lambda i: item_chunk[i] <= c)
            if h_qk is None:
                for other in others:
                    other.step()
            if h_pv is not None:
                o = _dot(vt_s[h_pv, :, ks], p)
                acc = o if acc is None else acc + o
            if h_qk is not None:
                for other in others:
                    other.step()
        vpu.finish()
        if h_pv is not None:
            denom = jnp.where(h_pv % 2 == 0, acc[MP - 1:MP], acc[0:1])
            ot_s[h_pv, :, qs] = acc * (1.0 / denom)
        if h_qk is not None:
            row_max = jnp.max(jnp.concatenate(top, axis=1), axis=0, keepdims=True)
            m_s[:, qs] = jnp.broadcast_to(row_max, (8, CQ))

    def head_step(h_qk, h_pv, h_next):
        ffn = _Spread(ffn_pieces(h_pv) if h_pv is not None else [], nq * nk)
        for j in range(nq):
            last = j + 1 == nq
            stage = _Spread(
                [part(stage_q, h_next if last else h_qk, pl.ds((j + 1) % nq * CQ, CQ), r, 8)
                 for r in range(0, LANES // 2, 8)], nk)
            attend(j * CQ, h_qk, h_pv, h_next if last else None, (stage, ffn))
            stage.finish()
        ffn.finish()

    def loop_body(h, carry):
        head_step(h + 1, h, jnp.minimum(h + 2, H - 1))
        return carry

    head_step(0, None, 1)
    lax.fori_loop(0, H - 1, loop_body, 0)

    def out_pieces(c):
        rows = pl.ds(out_off[c], OUT_CHUNKS[c])
        state = {}

        def gather():
            sub = lax.broadcasted_iota(jnp.int32, (8, OUT_CHUNKS[c]), 0)
            parts = []
            for h in range(0, H, 2):
                parts.append(ot_s[h, 0:16, rows])
                parts.append(jnp.where(sub < 4, ot_s[h, 16:24, rows], ot_s[h + 1, 0:8, rows]))
                parts.append(ot_s[h + 1, 8:24, rows])
            state["o"] = jnp.concatenate(parts, axis=0).astype(BF16).T

        def project(g):
            y = y_s[rows, tile(g)] + _dot(state["o"], wo_v[:, tile(g)])
            out_v[rows, tile(g)] = y.astype(out_v.dtype)

        return [gather] + [part(project, g) for g in range(G)] + [out_copy(c).start]

    work, c = ffn_pieces(H - 1), 0
    for j in range(nq):
        spread = _Spread(work, nk)
        attend(j * CQ, None, H - 1, others=(spread,))
        spread.finish()
        work = []
        while c < no and out_off[c] + OUT_CHUNKS[c] <= (j + 1) * CQ:
            work += out_pieces(c)
            c += 1
    for piece in work:
        piece()
    for c in range(no):
        out_copy(c).wait()


@jax.jit
def pallas_parallel_sum__mha_block__swiglu_ffn__prompt_kernel(
    A_x: jax.Array,
    A_wqkv: jax.Array,
    A_wo: jax.Array,
    B_x: jax.Array,
    B_w_gate: jax.Array,
    B_w_up: jax.Array,
    B_w_down: jax.Array,
):
    del B_x
    B, S, D = A_x.shape
    F = B_w_gate.shape[1]
    G = D // LANES
    assert B == 1 and D == 20 * H and S == sum(X_CHUNKS) == sum(OUT_CHUNKS)
    assert F % (FK * LANES) == 0
    any_spec = pl.BlockSpec(memory_space=pl.ANY)
    out = pl.pallas_call(
        _kernel,
        name="mha_swiglu",
        out_shape=jax.ShapeDtypeStruct((S, D), A_x.dtype),
        in_specs=[any_spec] * 6,
        out_specs=any_spec,
        scratch_shapes=[
            pltpu.VMEM((S, D), A_x.dtype),
            pltpu.VMEM((3, D, D), A_wqkv.dtype),
            pltpu.VMEM((D, D), A_wo.dtype),
            pltpu.VMEM((D, F), B_w_gate.dtype),
            pltpu.VMEM((D, F), B_w_up.dtype),
            pltpu.VMEM((F, D), B_w_down.dtype),
            pltpu.VMEM((S, D), A_x.dtype),
            pltpu.VMEM((2, D // 2, D), U32),
            pltpu.VMEM((S // 2, D), U32),
            pltpu.VMEM((2 * G - 1, S // 2, LANES), U32),
            pltpu.VMEM((2 * G - 1, LANES // 2, S), U32),
            pltpu.VMEM((LANES // 2, S), U32),
            pltpu.VMEM((H, MP, S), F32),
            pltpu.VMEM((H, MP, S), F32),
            pltpu.VMEM((S, S), F32),
            pltpu.VMEM((H, MP, S), F32),
            pltpu.VMEM((8, S), F32),
            pltpu.VMEM((S, D), F32),
            pltpu.VMEM((S // H // 2, F), U32),
            pltpu.VMEM((S // CK // VPU_EVERY, D // H, RK, LANES), F32),
            pltpu.SemaphoreType.DMA((len(X_CHUNKS) + 7 + len(OUT_CHUNKS),)),
        ],
        compiler_params=pltpu.CompilerParams(vmem_limit_bytes=110 * 2**20),
    )(A_x.reshape(S, D), A_wqkv, A_wo, B_w_gate, B_w_up, B_w_down)
    return out.reshape(B, S, D)
```

```python
import functools
import math

import jax
import jax.numpy as jnp
from jax import lax
import jax.experimental.pallas as pl
import jax.experimental.pallas.tpu as pltpu

H = 32
LANES = 128
F32 = jnp.float32
BF16 = jnp.bfloat16
U32 = jnp.uint32

X_CHUNKS = (320, 512, 512, 704)
OUT_CHUNKS = (256,) * 7 + (128, 128)
TK = 64
TQV = 1024
RQV = 64
TO = 64
CQ = 256
CK = 128
RK = 16
VPU_CHUNKS = (0, 1, 3, 4, 6, 8, 9, 11, 13)
MP = 24
FK = 4

NN = (((1,), (0,)), ((), ()))
NT = (((1,), (1,)), ((), ()))


def _dot(a, b, dims=NN):
    return lax.dot_general(a, b, dims, preferred_element_type=F32)


class _Spread:
    def __init__(self, items, slots, due=None):
        self.items = list(items)
        self.due = due or [i * slots // len(self.items) for i in range(len(self.items))]
        self.ready = lambda i: True
        self.done = self.tick = 0

    def step(self):
        while (self.done < len(self.items) and self.due[self.done] <= self.tick
               and self.ready(self.done)):
            self.items[self.done]()
            self.done += 1
        self.tick += 1

    def finish(self):
        for item in self.items[self.done:]:
            item()
        self.done = len(self.items)


def _kernel(x_hbm, wqkv_hbm, wo_hbm, wg_hbm, wu_hbm, wd_hbm, out_hbm,
            x_v, wqkv_v, wo_v, wg_v, wu_v, wd_v, out_v,
            wt_s, xn_s, kg_s, qg_s, qm_s, qf_s, vt_s, s_s, ot_s, m_s,
            y_s, hid_s, kb_s, sems):
    S, D = out_v.shape
    F = wg_v.shape[1]
    DH = D // H
    G = D // LANES
    TF = S // H
    nx, no, nq, nk = len(X_CHUNKS), len(OUT_CHUNKS), S // CQ, S // CK
    x_off = [sum(X_CHUNKS[:i]) for i in range(nx)]
    out_off = [sum(OUT_CHUNKS[:i]) for i in range(no)]
    q_scale = (DH ** -0.5) * math.log2(math.e)
    part = functools.partial

    def tile(g, n=1):
        return pl.ds(g * LANES, n * LANES)

    def aligned(start, size):
        return pl.ds(start if isinstance(start, int) else pl.multiple_of(start, size), size)

    def xn_block(i, size):
        return pltpu.bitcast(xn_s[aligned(i * (size // 2), size // 2), :], BF16)

    def x_copy(c):
        rows = pl.ds(x_off[c], X_CHUNKS[c])
        return pltpu.make_async_copy(x_hbm.at[rows, :], x_v.at[rows, :], sems.at[c])

    def w_copy(p):
        return pltpu.make_async_copy(
            wqkv_hbm.at[:, pl.ds(p * D, D)], wqkv_v.at[p], sems.at[nx + p])

    def out_copy(c):
        rows = pl.ds(out_off[c], OUT_CHUNKS[c])
        return pltpu.make_async_copy(
            out_v.at[rows, :], out_hbm.at[rows, :], sems.at[nx + 7 + c])

    late_copies = [
        pltpu.make_async_copy(src, dst, sems.at[nx + 3 + i]) for i, (src, dst) in
        enumerate(((wg_hbm, wg_v), (wu_hbm, wu_v), (wd_hbm, wd_v), (wo_hbm, wo_v)))]

    def layernorm(start, size):
        x = x_v[pl.ds(start, size), :].astype(F32)
        mean = jnp.sum(x, axis=-1, keepdims=True) * (1.0 / D)
        xc = x - mean
        var = jnp.sum(xc * xc, axis=-1, keepdims=True) * (1.0 / D)
        xn = (xc * lax.rsqrt(var + 1e-5)).astype(BF16)
        xn_s[pl.ds(start // 2, size // 2), :] = pltpu.bitcast(xn, U32)

    def project_k(i):
        rows = pl.ds(i * TK // 2, TK // 2)
        upper = lax.broadcasted_iota(jnp.int32, (TK // 2, LANES), 1) >= LANES // 2
        k = pltpu.bitcast(_dot(xn_block(i, TK), wqkv_v[1]).astype(BF16), U32)
        for g in range(G):
            kg = k[:, g * LANES:(g + 1) * LANES]
            kg_s[g, rows, :] = kg
            if g + 1 < G:
                kg_s[G + g, rows, :] = jnp.where(upper, kg, k[:, (g + 1) * LANES:(g + 2) * LANES])

    x_copy(0).start()
    w_copy(1).start()
    x_copy(0).wait()
    x_copy(1).start()
    layernorm(0, X_CHUNKS[0])
    w_copy(1).wait()
    for c in range(2, nx):
        x_copy(c).start()
    for c in range(nx):
        if c:
            x_copy(c).wait()
        if c == 1:
            w_copy(0).start()
            w_copy(2).start()
        if c + 1 == nx:
            w_copy(0).wait()
            w_copy(2).wait()
            for copy in late_copies:
                copy.start()
            for i, p in enumerate((0, 2)):
                wt_s[i] = pltpu.bitcast(wqkv_v[p].T, U32)
        for i in range(x_off[c] // TK, (x_off[c] + X_CHUNKS[c]) // TK):
            if i:
                project_k(i - 1)
            if c:
                layernorm(i * TK, TK)
    project_k(S // TK - 1)

    def head_group(h):
        start = h * DH
        straddles = start % LANES > LANES - DH
        if isinstance(h, int):
            return start // LANES + (G if straddles else 0)
        return jnp.where(straddles, G + start // LANES, start // LANES)

    def stage_q(h, cols, r0, n):
        row = lax.broadcasted_iota(jnp.int32, (n, cols.size), 0) + r0
        keep = ((row - h * (DH // 2)) & (LANES // 2 - 1)) < DH // 2
        rows = pl.ds(r0, n)
        qm_s[rows, cols] = jnp.where(keep, qg_s[head_group(h), rows, cols], U32(0))

    def splat_keys(h, chunk, slot):
        rows = pl.ds(((chunk + 1) * CK - RK) // 2, RK // 2)
        k = pltpu.bitcast(kg_s[head_group(h), rows, :], BF16).astype(F32)
        k = pltpu.roll(k, (LANES - (h * DH) % LANES) % LANES, 1)
        for d in range(DH):
            kb_s[slot, d] = jnp.broadcast_to(k[:, d:d + 1], (RK, LANES))

    def vpu_scores(h, slot, cols):
        acc = None
        for d in range(DH):
            term = kb_s[slot, d] * qf_s[h, pl.ds(d, 1), cols]
            acc = term if acc is None else acc + term
        return acc

    def project_qv(c, carry):
        cols = aligned(c * TQV, TQV)
        xn = xn_block(c, TQV)

        def project(i):
            return jnp.concatenate(
                [_dot(pltpu.bitcast(wt_s[i, r // 2:(r + RQV) // 2], BF16), xn, NT)
                 for r in range(0, D, RQV)], axis=0)

        q = (project(0) * q_scale).astype(BF16)
        qu = pltpu.bitcast(q, U32)
        full, half = LANES // 2, LANES // 4
        for g in range(G):
            qg_s[g, :, cols] = qu[g * full:(g + 1) * full]
            if g + 1 < G:
                qg_s[G + g, 0:half, cols] = qu[(g + 1) * full:(g + 1) * full + half]
                qg_s[G + g, half:full, cols] = qu[g * full + half:(g + 1) * full]
        qf = q.astype(F32)
        for h in range(H):
            qf_s[h, 0:DH, cols] = qf[h * DH:(h + 1) * DH]
        v = project(1).astype(BF16).astype(F32)
        sub = lax.broadcasted_iota(jnp.int32, (8, TQV), 0)
        for h in range(H):
            r0 = (h * DH) // 8 * 8
            if h % 2 == 0:
                vt_s[h, 0:16, cols] = v[r0:r0 + 16]
                vt_s[h, 16:24, cols] = jnp.where(sub < 4, v[r0 + 16:r0 + 24], 1.0)
            else:
                vt_s[h, 0:8, cols] = jnp.where(sub >= 4, v[r0:r0 + 8], 1.0)
                vt_s[h, 8:24, cols] = v[r0 + 8:r0 + 24]
        return carry

    for slot, chunk in enumerate(VPU_CHUNKS):
        splat_keys(0, chunk, slot)
    lax.fori_loop(0, S // TQV, project_qv, 0)
    stage_q(0, pl.ds(0, CQ), 0, LANES // 2)
    for copy in late_copies:
        copy.wait()

    def ffn_pieces(c):
        rows = aligned(c * TF, TF)
        state = {}

        def gate(n):
            state["gate"] = _dot(xn_block(c, TF), wg_v[:, tile(n)])

        def up(n):
            half = 0.5 * state["gate"]
            silu = half + half * jnp.tanh(half)
            hid = (silu * _dot(xn_block(c, TF), wu_v[:, tile(n)])).astype(BF16)
            hid_s[:, tile(n)] = pltpu.bitcast(hid, U32)

        def down(g, n):
            y = _dot(pltpu.bitcast(hid_s[:, tile(n, FK)], BF16), wd_v[tile(n, FK), tile(g)])
            state["y"] = state["y"] + y if n else x_v[rows, tile(g)].astype(F32) + y
            if n + FK == F // LANES:
                y_s[rows, tile(g)] = state["y"]

        pieces = [part(f, n) for n in range(F // LANES) for f in (gate, up)]
        return pieces + [part(down, g, n) for g in range(G) for n in range(0, F // LANES, FK)]

    def attend(q0, h_qk, h_pv, next_keys=None, others=()):
        qs = pl.ds(q0, CQ)
        tiles = CQ // LANES
        top = [None] * tiles
        items, item_chunk = [], []

        def update_max(t, value):
            top[t] = value if top[t] is None else jnp.maximum(top[t], value)

        def vpu_item(slot, chunk, t):
            cols = pl.ds(q0 + t * LANES, LANES)
            s = vpu_scores(h_qk, slot, cols)
            s_s[pl.ds((chunk + 1) * CK - RK, RK), cols] = s
            update_max(t, jnp.maximum(s[0:8], s[8:16]))
            if next_keys is not None and t + 1 == tiles:
                splat_keys(next_keys, chunk, slot)

        if h_qk is not None:
            group = head_group(h_qk)
            q = pltpu.bitcast(qm_s[:, qs], BF16)
            for slot, chunk in enumerate(VPU_CHUNKS):
                for t in range(tiles):
                    items.append(part(vpu_item, slot, chunk, t))
                    item_chunk.append(chunk)
        if h_pv is not None:
            m = m_s[:, qs]
            acc = None
        vpu = _Spread(items, 2 * nk - 1)

        for c in range(nk):
            ks = pl.ds(c * CK, CK)
            vpu.ready = lambda i: item_chunk[i] <= c
            if h_pv is not None:
                p = jnp.exp2(s_s[ks, qs].reshape(CK // 8, 8, CQ) - m[None]).reshape(CK, CQ)
            vpu.step()
            if h_qk is not None:
                n = CK - RK if c in VPU_CHUNKS else CK
                k = pltpu.bitcast(kg_s[group, pl.ds(c * CK // 2, n // 2), :], BF16)
                s = _dot(k, q)
                s_s[pl.ds(c * CK, n), qs] = s
                block_max = jnp.max(s.reshape(n // 8, 8, CQ), axis=0)
                for t in range(tiles):
                    update_max(t, block_max[:, t * LANES:(t + 1) * LANES])
            vpu.step()
            if h_qk is None:
                for other in others:
                    other.step()
            if h_pv is not None:
                o = _dot(vt_s[h_pv, :, ks], p)
                acc = o if acc is None else acc + o
            if h_qk is not None:
                for other in others:
                    other.step()
        vpu.finish()
        if h_pv is not None:
            denom = jnp.where(h_pv % 2 == 0, acc[MP - 1:MP], acc[0:1])
            ot_s[h_pv, :, qs] = acc * (1.0 / denom)
        if h_qk is not None:
            row_max = jnp.max(jnp.concatenate(top, axis=1), axis=0, keepdims=True)
            m_s[:, qs] = jnp.broadcast_to(row_max, (8, CQ))

    def head_step(h_qk, h_pv, h_next):
        pieces = ffn_pieces(h_pv) if h_pv is not None else []
        gaps = [13, 52] * (F // LANES) + [25] * (len(pieces) - 2 * F // LANES)
        due = [(2 * sum(gaps[:i]) + gap) * nq * nk // (2 * sum(gaps))
               for i, gap in enumerate(gaps)]
        ffn = _Spread(pieces, nq * nk, due)
        for j in range(nq):
            last = j + 1 == nq
            stage = _Spread(
                [part(stage_q, h_next if last else h_qk, pl.ds((j + 1) % nq * CQ, CQ), r, 8)
                 for r in range(0, LANES // 2, 8)], nk)
            attend(j * CQ, h_qk, h_pv, h_next if last else None, (stage, ffn))
            stage.finish()
        ffn.finish()

    def loop_body(h, carry):
        head_step(h + 1, h, jnp.minimum(h + 2, H - 1))
        return carry

    head_step(0, None, 1)
    lax.fori_loop(0, H - 1, loop_body, 0)

    def out_pieces(c):
        rows = pl.ds(out_off[c], OUT_CHUNKS[c])
        state = {}

        def gather():
            sub = lax.broadcasted_iota(jnp.int32, (8, OUT_CHUNKS[c]), 0)
            parts = []
            for h in range(0, H, 2):
                parts.append(ot_s[h, 0:16, rows])
                parts.append(jnp.where(sub < 4, ot_s[h, 16:24, rows], ot_s[h + 1, 0:8, rows]))
                parts.append(ot_s[h + 1, 8:24, rows])
            state["o"] = jnp.concatenate(parts, axis=0).astype(BF16).T

        def project(r, g):
            block = pl.ds(out_off[c] + r, TO)
            y = y_s[block, tile(g)] + _dot(state["o"][r:r + TO], wo_v[:, tile(g)])
            out_v[block, tile(g)] = y.astype(out_v.dtype)

        pieces = [part(project, r, g) for r in range(0, OUT_CHUNKS[c], TO) for g in range(G)]
        return [gather] + pieces + [out_copy(c).start]

    work = ffn_pieces(H - 1)
    needs = [0] * len(work)
    for c in range(no):
        work += out_pieces(c)
        needs += [out_off[c] + OUT_CHUNKS[c]] * (len(work) - len(needs))
    tail = _Spread(work, nq * nk * 13 // 10)
    for j in range(nq):
        tail.ready = lambda i: needs[i] <= j * CQ
        attend(j * CQ, None, H - 1, others=(tail,))
    tail.finish()
    for c in range(no):
        out_copy(c).wait()


@jax.jit
def pallas_parallel_sum__mha_block__swiglu_ffn__prompt_kernel(
    A_x: jax.Array,
    A_wqkv: jax.Array,
    A_wo: jax.Array,
    B_x: jax.Array,
    B_w_gate: jax.Array,
    B_w_up: jax.Array,
    B_w_down: jax.Array,
):
    del B_x
    B, S, D = A_x.shape
    F = B_w_gate.shape[1]
    G = D // LANES
    assert B == 1 and D == 20 * H and S == sum(X_CHUNKS) == sum(OUT_CHUNKS)
    assert F % (FK * LANES) == 0
    any_spec = pl.BlockSpec(memory_space=pl.ANY)
    out = pl.pallas_call(
        _kernel,
        name="mha_swiglu",
        out_shape=jax.ShapeDtypeStruct((S, D), A_x.dtype),
        in_specs=[any_spec] * 6,
        out_specs=any_spec,
        scratch_shapes=[
            pltpu.VMEM((S, D), A_x.dtype),
            pltpu.VMEM((3, D, D), A_wqkv.dtype),
            pltpu.VMEM((D, D), A_wo.dtype),
            pltpu.VMEM((D, F), B_w_gate.dtype),
            pltpu.VMEM((D, F), B_w_up.dtype),
            pltpu.VMEM((F, D), B_w_down.dtype),
            pltpu.VMEM((S, D), A_x.dtype),
            pltpu.VMEM((2, D // 2, D), U32),
            pltpu.VMEM((S // 2, D), U32),
            pltpu.VMEM((2 * G - 1, S // 2, LANES), U32),
            pltpu.VMEM((2 * G - 1, LANES // 2, S), U32),
            pltpu.VMEM((LANES // 2, S), U32),
            pltpu.VMEM((H, MP, S), F32),
            pltpu.VMEM((H, MP, S), F32),
            pltpu.VMEM((S, S), F32),
            pltpu.VMEM((H, MP, S), F32),
            pltpu.VMEM((8, S), F32),
            pltpu.VMEM((S, D), F32),
            pltpu.VMEM((S // H // 2, F), U32),
            pltpu.VMEM((len(VPU_CHUNKS), D // H, RK, LANES), F32),
            pltpu.SemaphoreType.DMA((len(X_CHUNKS) + 7 + len(OUT_CHUNKS),)),
        ],
        compiler_params=pltpu.CompilerParams(vmem_limit_bytes=110 * 2**20),
    )(A_x.reshape(S, D), A_wqkv, A_wo, B_w_gate, B_w_up, B_w_down)
    return out.reshape(B, S, D)
```
